```python
import jax
import jax.numpy as jnp

def _softmax(x, axis=-1):
    return jax.nn.softmax(x, axis=axis)
def _gelu(x):
    return jax.nn.gelu(x, approximate=True)
def _silu(x):
    return jax.nn.silu(x)
def _sigmoid(x):
    return jax.nn.sigmoid(x)
def _layernorm(x, axis=-1, eps=1e-5):
    m = jnp.mean(x, axis=axis, keepdims=True)
    v = jnp.var(x, axis=axis, keepdims=True)
    return (x - m) / jnp.sqrt(v + eps)
def _scatter_add(tgt, idx, src, axis=0):
    return tgt.at[idx].add(src)
def _segment_sum(src, seg, n):
    return jax.ops.segment_sum(src, seg, n)
class _Rng:
    def __init__(self, key):
        self._k = key
    def _next(self):
        self._k, sub = jax.random.split(self._k)
        return sub
    def normal(self, shape):
        return jax.random.normal(self._next(), shape, dtype=jnp.bfloat16)
    def randint(self, lo, hi, shape):
        return jax.random.randint(self._next(), shape, lo, hi, dtype=jnp.int32)
    def uniform(self, shape, lo=0.0, hi=1.0):
        return jax.random.uniform(self._next(), shape, jnp.bfloat16, lo, hi)
    def permutation(self, n):
        return jax.random.permutation(self._next(), n)


kernel_name = 'standalone__batchnorm__prompt'

def setup_inputs():
    _rng = _Rng(jax.random.key(int.from_bytes(__import__("os").urandom(4), "little")))
    _w = (lambda a: (lambda t: t.astype(jnp.bfloat16) if jnp.issubdtype(t.dtype, jnp.floating) else t)(jnp.asarray(a)))
    B, S, C = 2, 2048, 1024
    K = 3
    return {
        "x": _w((lambda *s: _rng.normal(s) * 0.05)(B, S, C)),
        "w": _w((lambda *s: _rng.normal(s) * 0.05)(K, C, C) * (1.0 / (K * C) ** 0.5)),
        "mean": _w((lambda *s: _rng.normal(s) * 0.05)(C) * 0.1),
        "var": _w(jnp.abs((lambda *s: _rng.normal(s) * 0.05)(C)) + 0.5),
        "g": _w((lambda *s: _rng.normal(s) * 0.05)(C) + 1.0),
        "b": _w((lambda *s: _rng.normal(s) * 0.05)(C) * 0.1),
    }

def reference(x, w, mean, var, g, b):
    K = 3
    P = K // 2
    S = x.shape[1]
    xp = jnp.pad(x, ((0, 0), (P, P), (0, 0)))
    y = sum(jnp.einsum('bsc,cd->bsd', xp[:, k:k + S, :], w[k]) for k in range(K))
    inv_std = 1.0 / jnp.sqrt(var + 1e-5)
    y = (y - mean) * (g * inv_std) + b
    return _silu(y)
```

```python
import functools

import jax
import jax.numpy as jnp
import jax.experimental.pallas as pl
import jax.experimental.pallas.tpu as pltpu

BF = jnp.bfloat16
F32 = jnp.float32
U32 = jnp.uint32
L = 128
PA, PB = 2.0 / 3.0, 1.5
CA = 1.0 / (2 * PA**2 * (PA**2 - PB**2))
CB = 1.0 / (PA**2 * 2 * PB**2 * (PB**2 - PA**2))
EPS = 1e-5


def _lo(u):
    return pltpu.unpack_elementwise(u, index=0, packed_dtype=BF, unpacked_dtype=F32)


def _hi(u):
    return pltpu.unpack_elementwise(u, index=1, packed_dtype=BF, unpacked_dtype=F32)


def _pack(lo, hi):
    return pltpu.pack_elementwise([lo, hi], packed_dtype=BF)


def _words(v):
    return pltpu.bitcast(v.astype(BF), U32)


def _spread(fs, nslots):
    out = [[] for _ in range(nslots)]
    for q, f in enumerate(fs):
        out[q * nslots // len(fs)].append(f)
    return out


def _conv_bn_silu(x, w, mean, var, g, b, *, R, GR=64, TR=64, KS=2, WA=2):
    B, S, C = x.shape
    n = R // 4
    nt = S // R
    T = B * nt
    KC = C // L
    XR = 16 + R + 32 + 16
    assert S % R == 0 and nt >= 2 and T >= 3 and n % TR == 0 and C % GR == 0

    def kernel(x_hbm, w_hbm, mean_ref, var_ref, g_ref, b_ref, o_hbm,
               xs, ts, wr, os_, xsem, wsem, osem, *gs):
        xu = xs.bitcast(U32)
        ou = os_.bitcast(U32)
        wu = wr.bitcast(U32)

        def tile_pos(t):
            bi = t // nt
            i = t % nt
            start = jnp.clip(i * R - 16, 0, S - R - 32)
            return bi, i, pl.multiple_of(start, 16)

        def x_copies(t, slot):
            bi, _, start = tile_pos(t)
            return [pltpu.make_async_copy(x_hbm.at[bi, pl.ds(start, R + 32), pl.ds(kc * L, L)],
                                          xs.at[slot, kc, pl.ds(16, R + 32), :], xsem.at[slot, kc])
                    for kc in range(KC)]

        def w_copies(nb):
            return [pltpu.make_async_copy(w_hbm.at[k, :, pl.ds(nb * L, L)], wr.at[k, nb], wsem.at[nb])
                    for k in range(3)]

        def o_copy(t, slot, nb):
            bi = t // nt
            i = t % nt
            return pltpu.make_async_copy(
                os_.at[slot, nb],
                o_hbm.at[bi, pl.ds(pl.multiple_of(i * R, R), R), pl.ds(nb * L, L)], osem.at[slot])

        def x_piece(t, slot, kc, j0, dep=None):
            _, i, start = tile_pos(t)
            off = pl.multiple_of((i * R - start) // 2, 8)
            xv = xu.at[slot, kc, pl.ds(off, R // 2 + 16), :]

            def ld(o):
                return xv[pl.ds(8 + 2 * j0 + o, TR, stride=2), :]
            we, wo, wp, wn = ld(0), ld(1), ld(-1), ld(2)
            d0, d1, d2, d3, d4, d5 = _hi(wp), _lo(we), _hi(we), _lo(wo), _hi(wo), _lo(wn)
            u = (PB * PB) * d2
            v = (PA * PA) * d2
            pa = d4 - u
            pb = d4 - v
            qa = PA * d3 - PB * d1
            qb = PB * d3 - PA * d1
            r = pl.ds(j0 // 2, TR // 2)
            ts[slot, 0, kc, r] = _words((d0 - u) + pb)
            ts[slot, 1, kc, r] = _words(pa + qa)
            ts[slot, 2, kc, r] = _words(pa - qa)
            ts[slot, 3, kc, r] = _words(pb + qb)
            ts[slot, 4, kc, r] = _words(pb - qb)
            ts[slot, 5, kc, r] = _words((d1 + d5) - (PA * PA + PB * PB) * d3)

        def x_pieces(t, slot, kc):
            return [functools.partial(x_piece, t, slot, kc, j0) for j0 in range(0, n, TR)]

        def g_piece(nb, r0, dep=None):
            r = pl.ds(r0 // 2, GR // 2)
            w0, w1, w2 = wu[0, nb, r], wu[1, nb, r], wu[2, nb, r]
            c2, c1 = PA * PA, PA
            if dep is not None:
                z = (pltpu.bitcast(dep[0:8, :], U32) >> 16) >> 16

                def cst(val):
                    c = pltpu.bitcast(pltpu.bitcast(jnp.full((8, L), val, F32), U32) | z, F32)
                    return jnp.tile(c, (GR // 16, 1))
                c2, c1 = cst(PA * PA), cst(PA)
            res = []
            for un in (_lo, _hi):
                g0, g1, g2 = un(w0), un(w1), un(w2)
                ea = g0 + g2 * c2
                eb = g0 * c2 + g2
                o = g1 * c1
                res.append((ea + o, ea - o, eb + o, eb - o))
            for q in range(4):
                gs[nb][q, r] = _pack(res[0][q], res[1][q])

        def g_pieces(nb):
            return [functools.partial(g_piece, nb, r0) for r0 in range(0, C, GR)]

        def rhs(i, nb, k0, kn):
            r = pl.ds(k0 // 2, kn // 2)
            words = wu[0, nb, r] if i == 0 else wu[2, nb, r] if i == 5 else gs[nb][i - 1, r]
            return pltpu.bitcast(words, BF)

        def step(slot, nb, scale, shift, side, ks):
            m = [None] * 6
            kw = KC // ks
            for q, i in enumerate((0, 5, 1, 2, 3, 4)):
                for kp in range(ks):
                    lhs = jnp.concatenate([pltpu.bitcast(ts[slot, i, kc], BF)
                                           for kc in range(kp * kw, (kp + 1) * kw)], axis=1)
                    d = jnp.dot(lhs, rhs(i, nb, kp * kw * L, kw * L), preferred_element_type=F32)
                    m[i] = d if kp == 0 else m[i] + d
                    for f in (side[q * ks + kp] if side else ()):
                        f(m[i])
            sc = scale[:, nb * L:(nb + 1) * L]
            sh = shift[:, nb * L:(nb + 1) * L]
            s1, e1 = m[1] + m[2], m[1] - m[2]
            s2, e2 = m[3] + m[4], m[3] - m[4]
            h0 = s1 * (sc * CA) + (s2 * (sc * CB) + (m[0] * sc + sh))
            h1 = e1 * (sc * (CA * PA)) + (e2 * (sc * (CB * PB)) + sh)
            h2 = s1 * (sc * (CA * PA**2)) + (s2 * (sc * (CB * PB**2)) + sh)
            h3 = e1 * (sc * (CA * PA**3)) + (e2 * (sc * (CB * PB**3)) + (m[5] * sc + sh))

            def act(h):
                return h * jnp.tanh(h) + h
            ou[slot, nb, pl.ds(0, n, stride=2), :] = _pack(act(h0), act(h1))
            ou[slot, nb, pl.ds(1, n, stride=2), :] = _pack(act(h2), act(h3))

        for c in w_copies(0):
            c.start()
        for c in x_copies(0, 0):
            c.start()
        for nb in range(1, WA + 1):
            for c in w_copies(nb):
                c.start(priority=1)
        zrows = jnp.zeros((16, L), BF)
        for s in range(2):
            for kc in range(KC):
                xs[s, kc, pl.ds(0, 16), :] = zrows
                xs[s, kc, pl.ds(XR - 16, 16), :] = zrows
        mean_v = mean_ref[...].astype(F32).reshape(1, C)
        var_v = var_ref[...].astype(F32).reshape(1, C)
        g_v = g_ref[...].astype(F32).reshape(1, C)
        b_v = b_ref[...].astype(F32).reshape(1, C)
        sc_full = g_v * (1.0 / jnp.sqrt(var_v + EPS))
        scale = 0.5 * sc_full
        shift = 0.5 * (b_v - mean_v * sc_full)

        for c in w_copies(0):
            c.wait()
        for f in g_pieces(0):
            f()
        for kc, c in enumerate(x_copies(0, 0)):
            c.wait()
            for f in x_pieces(0, 0, kc):
                f()

        def tile(t, first=False, last=False):
            slot = t % 2
            nslot = 1 - slot
            if not first:
                @pl.when(t >= 2)
                def _():
                    for nb in range(KC):
                        o_copy(t - 2, slot, nb).wait()
            if not first and not last:
                for c in x_copies(t + 1, nslot):
                    c.wait()

                @pl.when(t + 2 < T)
                def _():
                    for c in x_copies(t + 2, slot):
                        c.start()
            for nb in range(KC):
                if first:
                    def sync(dep=None, nb=nb):
                        if nb + 1 < KC:
                            for c in w_copies(nb + 1):
                                c.wait()
                        if nb + 1 + WA < KC:
                            for c in w_copies(nb + 1 + WA):
                                c.start(priority=1)
                        if nb + 1 + WA == KC - 1:
                            for c in x_copies(1, 1):
                                c.start(priority=1)
                        if nb + 1 + WA == KC:
                            for c in x_copies(2, 0):
                                c.start(priority=1)
                    side = [[] for _ in range(6 * KS)]
                    side[KS - 1].append(sync)
                    gp = g_pieces(nb + 1) if nb + 1 < KC else []
                    for q, f in enumerate(gp):
                        side[KS - 1 + q * (5 * KS) // len(gp)].append(f)
                elif last:
                    side = None
                else:
                    side = _spread(x_pieces(t + 1, nslot, nb), 6)
                step(slot, nb, scale, shift, side, KS if first else 1)
                o_copy(t, slot, nb).start()
            if first:
                for kc, c in enumerate(x_copies(1, 1)):
                    c.wait()
                    for f in x_pieces(1, 1, kc):
                        f()
            if last:
                for nb in range(KC):
                    o_copy(t - 1, nslot, nb).wait()
                for nb in range(KC):
                    o_copy(t, slot, nb).wait()

        tile(0, first=True)
        pl.loop(1, T - 1)(tile)
        tile(T - 1, last=True)

    vec = pl.BlockSpec((C,), lambda: (0,))
    hbm = pl.BlockSpec(memory_space=pl.ANY)
    return pl.pallas_call(
        kernel,
        in_specs=[hbm, hbm, vec, vec, vec, vec],
        out_specs=hbm,
        out_shape=jax.ShapeDtypeStruct((B, S, C), x.dtype),
        scratch_shapes=[
            pltpu.VMEM((2, KC, XR, L), BF),
            pltpu.VMEM((2, 6, KC, n // 2, L), U32),
            pltpu.VMEM((3, KC, C, L), BF),
            pltpu.VMEM((2, KC, R, L), BF),
            pltpu.SemaphoreType.DMA((2, KC)),
            pltpu.SemaphoreType.DMA((KC,)),
            pltpu.SemaphoreType.DMA((2,)),
        ] + [pltpu.VMEM((4, C // 2, L), U32) for _ in range(KC)],
        compiler_params=pltpu.CompilerParams(vmem_limit_bytes=100 * 1024 * 1024),
    )(x, w, mean, var, g, b)


@jax.jit
def pallas_standalone__batchnorm__prompt_kernel(
    x: jax.Array,
    w: jax.Array,
    mean: jax.Array,
    var: jax.Array,
    g: jax.Array,
    b: jax.Array,
):
    return _conv_bn_silu(x, w, mean, var, g, b, R=512)
```

```python
import functools

import jax
import jax.numpy as jnp
import jax.experimental.pallas as pl
import jax.experimental.pallas.tpu as pltpu

BF = jnp.bfloat16
F32 = jnp.float32
U32 = jnp.uint32
L = 128
PA, PB = 2.0 / 3.0, 1.5
CA = 1.0 / (2 * PA**2 * (PA**2 - PB**2))
CB = 1.0 / (PA**2 * 2 * PB**2 * (PB**2 - PA**2))
EPS = 1e-5


def _lo(u):
    return pltpu.unpack_elementwise(u, index=0, packed_dtype=BF, unpacked_dtype=F32)


def _hi(u):
    return pltpu.unpack_elementwise(u, index=1, packed_dtype=BF, unpacked_dtype=F32)


def _pack(lo, hi):
    return pltpu.pack_elementwise([lo, hi], packed_dtype=BF)


def _words(v):
    return pltpu.bitcast(v.astype(BF), U32)


def _spread(fs, nslots):
    out = [[] for _ in range(nslots)]
    for q, f in enumerate(fs):
        out[q * nslots // len(fs)].append(f)
    return out


def _conv_bn_silu(x, w, mean, var, g, b, *, R=512, GR=64, TR=64, H=2):
    B, S, C = x.shape
    n = R // 4
    nt = S // R
    T = B * nt
    KC = C // L
    XR = 16 + R + 32 + 16
    assert S % R == 0 and nt >= 2 and T >= 3 and n % TR == 0 and C % GR == 0
    assert KC >= 4 and 1 <= H < KC

    def kernel(x_hbm, w_hbm, mean_ref, var_ref, g_ref, b_ref, o_hbm,
               xs, ts, wr, os_, os0, xsem0, xsem, wsem, osem, *gs):
        xu = xs.bitcast(U32)
        wu = wr.bitcast(U32)

        def tile_pos(t):
            bi = t // nt
            i = t % nt
            start = jnp.clip(i * R - 16, 0, S - R - 32)
            return bi, i, pl.multiple_of(start, 16)

        def x_copies(t, slot, per_block_sem=False):
            bi, _, start = tile_pos(t)
            return [pltpu.make_async_copy(x_hbm.at[bi, pl.ds(start, R + 32), pl.ds(kc * L, L)],
                                          xs.at[slot, kc, pl.ds(16, R + 32), :],
                                          xsem0.at[slot, kc] if per_block_sem else xsem.at[slot])
                    for kc in range(KC)]

        def x_wait_all(slot):
            win = xs.at[slot, :, pl.ds(16, R + 32), :]
            pltpu.make_async_copy(win, win, xsem.at[slot]).wait()

        def w_copies(nb):
            return [pltpu.make_async_copy(w_hbm.at[k, :, pl.ds(nb * L, L)], wr.at[k, nb], wsem.at[nb])
                    for k in range(3)]

        def o_stage(oslot, nb):
            return os0.at[nb] if (isinstance(oslot, int) and oslot == 2) else os_.at[oslot, nb]

        def o_copy(t, oslot, nb):
            bi = t // nt
            i = t % nt
            return pltpu.make_async_copy(
                o_stage(oslot, nb),
                o_hbm.at[bi, pl.ds(pl.multiple_of(i * R, R), R), pl.ds(nb * L, L)], osem.at[oslot])

        def o_wait_all(oslot):
            pltpu.make_async_copy(os_.at[oslot], os_.at[oslot], osem.at[oslot]).wait()

        def x_piece(t, slot, kc, j0, dep=None):
            _, i, start = tile_pos(t)
            off = pl.multiple_of((i * R - start) // 2, 8)
            xv = xu.at[slot, kc, pl.ds(off, R // 2 + 16), :]

            def ld(o):
                return xv[pl.ds(8 + 2 * j0 + o, TR, stride=2), :]
            we, wo, wp, wn = ld(0), ld(1), ld(-1), ld(2)
            d0, d1, d2, d3, d4, d5 = _hi(wp), _lo(we), _hi(we), _lo(wo), _hi(wo), _lo(wn)
            u = (PB * PB) * d2
            v = (PA * PA) * d2
            pa = d4 - u
            pb = d4 - v
            qa = PA * d3 - PB * d1
            qb = PB * d3 - PA * d1
            r = pl.ds(j0 // 2, TR // 2)
            ts[slot, 0, kc, r] = _words((d0 - u) + pb)
            ts[slot, 1, kc, r] = _words(pa + qa)
            ts[slot, 2, kc, r] = _words(pa - qa)
            ts[slot, 3, kc, r] = _words(pb + qb)
            ts[slot, 4, kc, r] = _words(pb - qb)
            ts[slot, 5, kc, r] = _words((d1 + d5) - (PA * PA + PB * PB) * d3)

        def x_pieces(t, slot, kc):
            return [functools.partial(x_piece, t, slot, kc, j0) for j0 in range(0, n, TR)]

        def g_piece(nb, r0, dep=None):
            r = pl.ds(r0 // 2, GR // 2)
            w0, w1, w2 = wu[0, nb, r], wu[1, nb, r], wu[2, nb, r]
            c2, c1 = PA * PA, PA
            if dep is not None:
                z = (pltpu.bitcast(dep[0:8, :], U32) >> 16) >> 16

                def cst(val):
                    c = pltpu.bitcast(pltpu.bitcast(jnp.full((8, L), val, F32), U32) | z, F32)
                    return jnp.tile(c, (GR // 16, 1))
                c2, c1 = cst(PA * PA), cst(PA)
            res = []
            for un in (_lo, _hi):
                g0, g1, g2 = un(w0), un(w1), un(w2)
                ea = g0 + g2 * c2
                eb = g0 * c2 + g2
                o = g1 * c1
                res.append((ea + o, ea - o, eb + o, eb - o))
            for q in range(4):
                gs[nb][q, r] = _pack(res[0][q], res[1][q])

        def g_pieces(nb):
            return [functools.partial(g_piece, nb, r0) for r0 in range(0, C, GR)]

        def step(slot, oslot, nb, scale, shift, side=None, order=(0, 1, 2, 3, 4, 5)):
            m = [None] * 6
            for q, i in enumerate(order):
                lhs = jnp.concatenate([pltpu.bitcast(ts[slot, i, kc], BF) for kc in range(KC)], axis=1)
                words = wu[0, nb] if i == 0 else wu[2, nb] if i == 5 else gs[nb][i - 1]
                m[i] = jnp.dot(lhs, pltpu.bitcast(words, BF), preferred_element_type=F32)
                for f in (side[q] if side else ()):
                    f(m[i])
            sc = scale[:, nb * L:(nb + 1) * L]
            sh = shift[:, nb * L:(nb + 1) * L]
            s1, e1 = m[1] + m[2], m[1] - m[2]
            s2, e2 = m[3] + m[4], m[3] - m[4]
            h0 = s1 * (sc * CA) + (s2 * (sc * CB) + (m[0] * sc + sh))
            h1 = e1 * (sc * (CA * PA)) + (e2 * (sc * (CB * PB)) + sh)
            h2 = s1 * (sc * (CA * PA**2)) + (s2 * (sc * (CB * PB**2)) + sh)
            h3 = e1 * (sc * (CA * PA**3)) + (e2 * (sc * (CB * PB**3)) + (m[5] * sc + sh))

            def act(h):
                return h * jnp.tanh(h) + h
            ov = (os0.bitcast(U32).at[nb] if (isinstance(oslot, int) and oslot == 2)
                  else os_.bitcast(U32).at[oslot, nb])
            ov[pl.ds(0, n, stride=2), :] = _pack(act(h0), act(h1))
            ov[pl.ds(1, n, stride=2), :] = _pack(act(h2), act(h3))

        x0 = x_copies(0, 0, True)
        x1 = x_copies(1, 1, True)
        for c in w_copies(0) + x0:
            c.start()
        for nb in (1, 2):
            for c in w_copies(nb):
                c.start(priority=1)
        zrows = jnp.zeros((16, L), BF)
        for s in range(2):
            for kc in range(KC):
                xs[s, kc, pl.ds(0, 16), :] = zrows
                xs[s, kc, pl.ds(XR - 16, 16), :] = zrows
        mean_v = mean_ref[...].astype(F32).reshape(1, C)
        var_v = var_ref[...].astype(F32).reshape(1, C)
        g_v = g_ref[...].astype(F32).reshape(1, C)
        b_v = b_ref[...].astype(F32).reshape(1, C)
        sc_full = g_v * (1.0 / jnp.sqrt(var_v + EPS))
        scale = 0.5 * sc_full
        shift = 0.5 * (b_v - mean_v * sc_full)

        for c in w_copies(0):
            c.wait()
        for f in g_pieces(0):
            f()
        for kc in range(KC):
            x0[kc].wait()
            for f in x_pieces(0, 0, kc):
                f()

        slots = [[] for _ in range(6 * KC)]
        for nb in range(1, KC):
            def sync(dep=None, nb=nb):
                for c in w_copies(nb):
                    c.wait()
                if nb + 2 < KC:
                    for c in w_copies(nb + 2):
                        c.start(priority=1)
                if nb + 2 == KC:
                    for c in x1:
                        c.start(priority=1)
                if nb + 1 == KC:
                    for c in x_copies(2, 0):
                        c.start(priority=1)
            d0 = 6 * nb - 2
            slots[d0].append(sync)
            for q, fs in enumerate(_spread(g_pieces(nb), 4)):
                slots[d0 + q] += fs
        for nb in range(KC):
            step(0, 2 if nb < H else 0, nb, scale, shift, slots[6 * nb:6 * nb + 6], (0, 5, 1, 2, 3, 4))
        for nb in range(KC):
            o_copy(0, 2 if nb < H else 0, nb).start()
        for kc in range(KC):
            x1[kc].wait()
            for f in x_pieces(1, 1, kc):
                f()
        for nb in range(H):
            step(1, 0, nb, scale, shift)
            o_copy(1, 0, nb).start()

        def body(t, last=False):
            slot = t % 2
            nslot = 1 - slot
            if not last:
                x_wait_all(nslot)
                pieces = _spread([f for kc in range(KC) for f in x_pieces(t + 1, nslot, kc)], KC - H)
            for nb in range(H, KC):
                side = None
                if not last:
                    fs = list(pieces[nb - H])
                    if nb == min(H + 2, KC - 1):
                        def prefetch(dep=None):
                            for c in x_copies(jnp.minimum(t + 2, T - 1), slot):
                                c.start()
                        fs = [prefetch] + fs
                    side = _spread(fs, 6)
                step(slot, slot, nb, scale, shift, side)
                o_copy(t, slot, nb).start()
            if not last:
                for nb in range(H):
                    step(nslot, slot, nb, scale, shift)
                    o_copy(t + 1, slot, nb).start()
                o_wait_all(nslot)

        pl.loop(1, T - 1)(body)
        body(T - 1, last=True)
        x_wait_all(T % 2)
        for nb in range(H):
            o_copy(0, 2, nb).wait()
        o_wait_all(T % 2)
        for nb in range(H, KC):
            o_copy(T - 1, (T - 1) % 2, nb).wait()

    vec = pl.BlockSpec((C,), lambda: (0,))
    hbm = pl.BlockSpec(memory_space=pl.ANY)
    return pl.pallas_call(
        kernel,
        in_specs=[hbm, hbm, vec, vec, vec, vec],
        out_specs=hbm,
        out_shape=jax.ShapeDtypeStruct((B, S, C), x.dtype),
        scratch_shapes=[
            pltpu.VMEM((2, KC, XR, L), BF),
            pltpu.VMEM((2, 6, KC, n // 2, L), U32),
            pltpu.VMEM((3, KC, C, L), BF),
            pltpu.VMEM((2, KC, R, L), BF),
            pltpu.VMEM((H, R, L), BF),
            pltpu.SemaphoreType.DMA((2, KC)),
            pltpu.SemaphoreType.DMA((2,)),
            pltpu.SemaphoreType.DMA((KC,)),
            pltpu.SemaphoreType.DMA((3,)),
        ] + [pltpu.VMEM((4, C // 2, L), U32) for _ in range(KC)],
        compiler_params=pltpu.CompilerParams(vmem_limit_bytes=100 * 1024 * 1024,
                                             disable_bounds_checks=True),
    )(x, w, mean, var, g, b)


@jax.jit
def pallas_standalone__batchnorm__prompt_kernel(
    x: jax.Array,
    w: jax.Array,
    mean: jax.Array,
    var: jax.Array,
    g: jax.Array,
    b: jax.Array,
):
    return _conv_bn_silu(x, w, mean, var, g, b)
```

```python
import functools

import jax
import jax.numpy as jnp
import jax.experimental.pallas as pl
import jax.experimental.pallas.tpu as pltpu

BF = jnp.bfloat16
F32 = jnp.float32
U32 = jnp.uint32
L = 128
PA, PB = 2.0 / 3.0, 1.5
CA = 1.0 / (2 * PA**2 * (PA**2 - PB**2))
CB = 1.0 / (PA**2 * 2 * PB**2 * (PB**2 - PA**2))
EPS = 1e-5


def _lo(u):
    return pltpu.bitcast(u << 16, F32)


def _hi(u):
    return pltpu.bitcast(u & jnp.uint32(0xFFFF0000), F32)


def _pair(lo, hi):
    def rounded(v):
        return pltpu.bitcast(v.astype(BF).astype(F32), U32)
    return (rounded(lo) >> 16) | rounded(hi)


def _words(v):
    return pltpu.bitcast(v.astype(BF), U32)


def _spread(fs, nslots):
    out = [[] for _ in range(nslots)]
    for q, f in enumerate(fs):
        out[q * nslots // len(fs)].append(f)
    return out


def _conv_bn_silu(x, w, mean, var, g, b, *, R=512, GR=64, TR=64, H=2):
    B, S, C = x.shape
    n = R // 4
    nt = S // R
    T = B * nt
    KC = C // L
    XR = 16 + R + 32 + 16
    assert S % R == 0 and nt >= 2 and T >= 3 and n % TR == 0 and C % GR == 0
    assert KC >= 4 and 1 <= H < KC

    def kernel(x_hbm, w_hbm, mean_ref, var_ref, g_ref, b_ref, o_hbm,
               xs, ts, wr, os_, os0, xsem0, xsem, wsem, osem, *gs):
        xu = xs.bitcast(U32)
        wu = wr.bitcast(U32)

        def tile_pos(t):
            bi = t // nt
            i = t % nt
            start = jnp.clip(i * R - 16, 0, S - R - 32)
            return bi, i, pl.multiple_of(start, 16)

        def x_copies(t, slot, per_block_sem=False):
            bi, _, start = tile_pos(t)
            return [pltpu.make_async_copy(x_hbm.at[bi, pl.ds(start, R + 32), pl.ds(kc * L, L)],
                                          xs.at[slot, kc, pl.ds(16, R + 32), :],
                                          xsem0.at[slot, kc] if per_block_sem else xsem.at[slot])
                    for kc in range(KC)]

        def x_wait_all(slot):
            win = xs.at[slot, :, pl.ds(16, R + 32), :]
            pltpu.make_async_copy(win, win, xsem.at[slot]).wait()

        def w_copies(nb):
            return [pltpu.make_async_copy(w_hbm.at[k, :, pl.ds(nb * L, L)], wr.at[k, nb], wsem.at[nb])
                    for k in range(3)]

        def o_stage(oslot, nb):
            return (os0.at[nb, pl.ds(0, R), :] if (isinstance(oslot, int) and oslot == 2)
                    else os_.at[oslot, nb, pl.ds(0, R), :])

        def o_copy(t, oslot, nb):
            bi = t // nt
            i = t % nt
            return pltpu.make_async_copy(
                o_stage(oslot, nb),
                o_hbm.at[bi, pl.ds(pl.multiple_of(i * R, R), R), pl.ds(nb * L, L)], osem.at[oslot])

        def o_wait_all(oslot):
            blocks = os_.at[oslot, :, pl.ds(0, R), :]
            pltpu.make_async_copy(blocks, blocks, osem.at[oslot]).wait()

        def x_piece(t, slot, kc, j0, dep=None):
            _, i, start = tile_pos(t)
            off = pl.multiple_of((i * R - start) // 2, 8)
            xv = xu.at[slot, kc, pl.ds(off, R // 2 + 16), :]

            def ld(o):
                return xv[pl.ds(8 + 2 * j0 + o, TR, stride=2), :]
            we, wo, wp, wn = ld(0), ld(1), ld(-1), ld(2)
            d0, d1, d2, d3, d4, d5 = _hi(wp), _lo(we), _hi(we), _lo(wo), _hi(wo), _lo(wn)
            u = (PB * PB) * d2
            v = (PA * PA) * d2
            pa = d4 - u
            pb = d4 - v
            qa = PA * d3 - PB * d1
            qb = PB * d3 - PA * d1
            r = pl.ds(j0 // 2, TR // 2)
            ts[slot, 0, kc, r] = _words((d0 - u) + pb)
            ts[slot, 1, kc, r] = _words(pa + qa)
            ts[slot, 2, kc, r] = _words(pa - qa)
            ts[slot, 3, kc, r] = _words(pb + qb)
            ts[slot, 4, kc, r] = _words(pb - qb)
            ts[slot, 5, kc, r] = _words((d1 + d5) - (PA * PA + PB * PB) * d3)

        def x_pieces(t, slot, kc):
            return [functools.partial(x_piece, t, slot, kc, j0) for j0 in range(0, n, TR)]

        def g_piece(nb, r0, dep=None):
            r = pl.ds(r0, GR)
            g0, g1, g2 = (wr[k, nb, r].astype(F32) for k in range(3))
            c2, c1 = PA * PA, PA
            if dep is not None:
                z = (pltpu.bitcast(dep[0:8, :], U32) >> 16) >> 16

                def cst(val):
                    c = pltpu.bitcast(pltpu.bitcast(jnp.full((8, L), val, F32), U32) | z, F32)
                    return jnp.tile(c, (GR // 8, 1))
                c2, c1 = cst(PA * PA), cst(PA)
            ea = g0 + g2 * c2
            eb = g0 * c2 + g2
            o = g1 * c1
            gs[nb][0, r] = (ea + o).astype(BF)
            gs[nb][1, r] = (ea - o).astype(BF)
            gs[nb][2, r] = (eb + o).astype(BF)
            gs[nb][3, r] = (eb - o).astype(BF)

        def g_pieces(nb):
            return [functools.partial(g_piece, nb, r0) for r0 in range(0, C, GR)]

        def step(slot, oslot, nb, scale, shift, side=None, order=(0, 1, 2, 3, 4, 5)):
            m = [None] * 6
            for q, i in enumerate(order):
                lhs = jnp.concatenate([pltpu.bitcast(ts[slot, i, kc], BF) for kc in range(KC)], axis=1)
                words = wu[0, nb] if i == 0 else wu[2, nb] if i == 5 else gs[nb].bitcast(U32)[i - 1]
                m[i] = jnp.dot(lhs, pltpu.bitcast(words, BF), preferred_element_type=F32)
                for f in (side[q] if side else ()):
                    f(m[i])
            sc = scale[:, nb * L:(nb + 1) * L]
            sh = shift[:, nb * L:(nb + 1) * L]
            s1, e1 = m[1] + m[2], m[1] - m[2]
            s2, e2 = m[3] + m[4], m[3] - m[4]
            h0 = s1 * (sc * CA) + (s2 * (sc * CB) + (m[0] * sc + sh))
            h1 = e1 * (sc * (CA * PA)) + (e2 * (sc * (CB * PB)) + sh)
            h2 = s1 * (sc * (CA * PA**2)) + (s2 * (sc * (CB * PB**2)) + sh)
            h3 = e1 * (sc * (CA * PA**3)) + (e2 * (sc * (CB * PB**3)) + (m[5] * sc + sh))

            def act(h):
                return h * jnp.tanh(h) + h
            ov = (os0.bitcast(U32).at[nb] if (isinstance(oslot, int) and oslot == 2)
                  else os_.bitcast(U32).at[oslot, nb])
            ov[pl.ds(0, n, stride=2), :] = _pair(act(h0), act(h1))
            ov[pl.ds(1, n, stride=2), :] = _pair(act(h2), act(h3))

        zrows = jnp.zeros((16, L), BF)
        for s in range(2):
            for kc in range(KC):
                xs[s, kc, pl.ds(0, 16), :] = zrows
                xs[s, kc, pl.ds(XR - 16, 16), :] = zrows
        x0 = x_copies(0, 0, True)
        x1 = x_copies(1, 1, True)
        for c in w_copies(0) + x0:
            c.start()
        for nb in (1, 2):
            for c in w_copies(nb):
                c.start(priority=1)
        mean_v = mean_ref[...].astype(F32).reshape(1, C)
        var_v = var_ref[...].astype(F32).reshape(1, C)
        g_v = g_ref[...].astype(F32).reshape(1, C)
        b_v = b_ref[...].astype(F32).reshape(1, C)
        sc_full = g_v * (1.0 / jnp.sqrt(var_v + EPS))
        scale = 0.5 * sc_full
        shift = 0.5 * (b_v - mean_v * sc_full)

        for c in w_copies(0):
            c.wait()
        for f in g_pieces(0):
            f()
        for kc in range(KC):
            x0[kc].wait()
            for f in x_pieces(0, 0, kc):
                f()

        slots = [[] for _ in range(6 * KC)]
        for nb in range(1, KC):
            def sync(dep=None, nb=nb):
                for c in w_copies(nb):
                    c.wait()
                if nb + 2 < KC:
                    for c in w_copies(nb + 2):
                        c.start(priority=1)
                if nb + 2 == KC:
                    for c in x1:
                        c.start(priority=1)
                if nb + 1 == KC:
                    for c in x_copies(2, 0):
                        c.start(priority=1)
            d0 = 6 * nb - 2
            slots[d0].append(sync)
            for q, fs in enumerate(_spread(g_pieces(nb), 4)):
                slots[d0 + q] += fs
        for nb in range(KC):
            step(0, 2 if nb < H else 0, nb, scale, shift, slots[6 * nb:6 * nb + 6], (0, 5, 1, 2, 3, 4))
        for nb in range(KC):
            o_copy(0, 2 if nb < H else 0, nb).start()
        for kc in range(KC):
            x1[kc].wait()
            for f in x_pieces(1, 1, kc):
                f()
        for nb in range(H):
            step(1, 0, nb, scale, shift)
            o_copy(1, 0, nb).start()

        def body(t, last=False):
            slot = t % 2
            nslot = 1 - slot
            if not last:
                x_wait_all(nslot)
                pieces = _spread([f for kc in range(KC) for f in x_pieces(t + 1, nslot, kc)], KC - H)
            for nb in range(H, KC):
                side = None
                if not last:
                    fs = list(pieces[nb - H])
                    if nb == min(H + 2, KC - 1):
                        def prefetch(dep=None):
                            for c in x_copies(jnp.minimum(t + 2, T - 1), slot):
                                c.start()
                        fs = [prefetch] + fs
                    side = _spread(fs, 6)
                step(slot, slot, nb, scale, shift, side)
                o_copy(t, slot, nb).start()
            if not last:
                for nb in range(H):
                    step(nslot, slot, nb, scale, shift)
                    o_copy(t + 1, slot, nb).start()
                o_wait_all(nslot)

        pl.loop(1, T - 1)(body)
        body(T - 1, last=True)
        x_wait_all(T % 2)
        for nb in range(H):
            o_copy(0, 2, nb).wait()
        o_wait_all(T % 2)
        for nb in range(H, KC):
            o_copy(T - 1, (T - 1) % 2, nb).wait()

    vec = pl.BlockSpec((C,), lambda: (0,))
    hbm = pl.BlockSpec(memory_space=pl.ANY)
    return pl.pallas_call(
        kernel,
        in_specs=[hbm, hbm, vec, vec, vec, vec],
        out_specs=hbm,
        out_shape=jax.ShapeDtypeStruct((B, S, C), x.dtype),
        scratch_shapes=[
            pltpu.VMEM((2, KC, XR, L), BF),
            pltpu.VMEM((2, 6, KC, n // 2, L), U32),
            pltpu.VMEM((3, KC, C, L), BF),
            pltpu.VMEM((2, KC, R + 16, L), BF),
            pltpu.VMEM((H, R + 16, L), BF),
            pltpu.SemaphoreType.DMA((2, KC)),
            pltpu.SemaphoreType.DMA((2,)),
            pltpu.SemaphoreType.DMA((KC,)),
            pltpu.SemaphoreType.DMA((3,)),
        ] + [pltpu.VMEM((4, C, L), BF) for _ in range(KC)],
        compiler_params=pltpu.CompilerParams(vmem_limit_bytes=100 * 1024 * 1024,
                                             disable_bounds_checks=True),
    )(x, w, mean, var, g, b)


@jax.jit
def pallas_standalone__batchnorm__prompt_kernel(
    x: jax.Array,
    w: jax.Array,
    mean: jax.Array,
    var: jax.Array,
    g: jax.Array,
    b: jax.Array,
):
    return _conv_bn_silu(x, w, mean, var, g, b)
```

```python
import functools

import jax
import jax.numpy as jnp
import jax.experimental.pallas as pl
import jax.experimental.pallas.tpu as pltpu

BF = jnp.bfloat16
F32 = jnp.float32
U32 = jnp.uint32
L = 128
PA, PB = 2.0 / 3.0, 1.5
CA = 1.0 / (2 * PA**2 * (PA**2 - PB**2))
CB = 1.0 / (PA**2 * 2 * PB**2 * (PB**2 - PA**2))
EPS = 1e-5


def _lo(u):
    return pltpu.bitcast(u << 16, F32)


def _hi(u):
    return pltpu.bitcast(u & jnp.uint32(0xFFFF0000), F32)


def _pair(lo, hi):
    def rounded(v):
        return pltpu.bitcast(v.astype(BF).astype(F32), U32)
    return (rounded(lo) >> 16) | rounded(hi)


def _words(v):
    return pltpu.bitcast(v.astype(BF), U32)


def _spread(fs, nslots):
    out = [[] for _ in range(nslots)]
    for q, f in enumerate(fs):
        out[q * nslots // len(fs)].append(f)
    return out


def _conv_bn_silu(x, w, mean, var, g, b, *, R=512, GR=32, TR=64, H=2):
    B, S, C = x.shape
    n = R // 4
    nt = S // R
    T = B * nt
    KC = C // L
    XR = 16 + R + 32 + 16
    assert S % R == 0 and nt >= 2 and T >= 3 and n % TR == 0 and C % GR == 0
    assert KC >= 4 and 1 <= H < KC

    def kernel(x_hbm, w_hbm, mean_ref, var_ref, g_ref, b_ref, o_hbm,
               xs, ts, wr, os_, os0, xsem0, xsem, wsem, osem, *gs):
        xu = xs.bitcast(U32)
        wu = wr.bitcast(U32)

        def tile_pos(t):
            bi = t // nt
            i = t % nt
            start = jnp.clip(i * R - 16, 0, S - R - 32)
            return bi, i, pl.multiple_of(start, 16)

        def x_copies(t, slot, per_block_sem=False):
            bi, _, start = tile_pos(t)
            return [pltpu.make_async_copy(x_hbm.at[bi, pl.ds(start, R + 32), pl.ds(kc * L, L)],
                                          xs.at[slot, kc, pl.ds(16, R + 32), :],
                                          xsem0.at[slot, kc] if per_block_sem else xsem.at[slot])
                    for kc in range(KC)]

        def x_wait_all(slot):
            win = xs.at[slot, :, pl.ds(16, R + 32), :]
            pltpu.make_async_copy(win, win, xsem.at[slot]).wait()

        def w_copies(nb):
            return [pltpu.make_async_copy(w_hbm.at[k, :, pl.ds(nb * L, L)], wr.at[k, nb], wsem.at[nb])
                    for k in range(3)]

        def o_stage(oslot, nb):
            return (os0.at[nb, pl.ds(0, R), :] if (isinstance(oslot, int) and oslot == 2)
                    else os_.at[oslot, nb, pl.ds(0, R), :])

        def o_copy(t, oslot, nb):
            bi = t // nt
            i = t % nt
            return pltpu.make_async_copy(
                o_stage(oslot, nb),
                o_hbm.at[bi, pl.ds(pl.multiple_of(i * R, R), R), pl.ds(nb * L, L)], osem.at[oslot])

        def o_wait_all(oslot):
            blocks = os_.at[oslot, :, pl.ds(0, R), :]
            pltpu.make_async_copy(blocks, blocks, osem.at[oslot]).wait()

        def x_piece(t, slot, kc, j0, dep=None):
            _, i, start = tile_pos(t)
            off = pl.multiple_of((i * R - start) // 2, 8)
            xv = xu.at[slot, kc, pl.ds(off, R // 2 + 16), :]

            def ld(o):
                return xv[pl.ds(8 + 2 * j0 + o, TR, stride=2), :]
            we, wo, wp, wn = ld(0), ld(1), ld(-1), ld(2)
            d0, d1, d2, d3, d4, d5 = _hi(wp), _lo(we), _hi(we), _lo(wo), _hi(wo), _lo(wn)
            u = (PB * PB) * d2
            v = (PA * PA) * d2
            pa = d4 - u
            pb = d4 - v
            qa = PA * d3 - PB * d1
            qb = PB * d3 - PA * d1
            r = pl.ds(j0 // 2, TR // 2)
            ts[slot, 0, kc, r] = _words((d0 - u) + pb)
            ts[slot, 1, kc, r] = _words(pa + qa)
            ts[slot, 2, kc, r] = _words(pa - qa)
            ts[slot, 3, kc, r] = _words(pb + qb)
            ts[slot, 4, kc, r] = _words(pb - qb)
            ts[slot, 5, kc, r] = _words((d1 + d5) - (PA * PA + PB * PB) * d3)

        def x_pieces(t, slot, kc):
            return [functools.partial(x_piece, t, slot, kc, j0) for j0 in range(0, n, TR)]

        def g_piece(nb, r0, dep=None):
            r = pl.ds(r0, GR)
            g0, g1, g2 = (wr[k, nb, r].astype(F32) for k in range(3))
            c2, c1 = PA * PA, PA
            if dep is not None:
                z = (pltpu.bitcast(dep[0:8, :], U32) >> 16) >> 16

                def cst(val):
                    c = pltpu.bitcast(pltpu.bitcast(jnp.full((8, L), val, F32), U32) | z, F32)
                    return jnp.tile(c, (GR // 8, 1))
                c2, c1 = cst(PA * PA), cst(PA)
            ea = g0 + g2 * c2
            eb = g0 * c2 + g2
            o = g1 * c1
            gs[nb][0, r] = (ea + o).astype(BF)
            gs[nb][1, r] = (ea - o).astype(BF)
            gs[nb][2, r] = (eb + o).astype(BF)
            gs[nb][3, r] = (eb - o).astype(BF)

        def g_pieces(nb):
            return [functools.partial(g_piece, nb, r0) for r0 in range(0, C, GR)]

        def step(slot, oslot, nb, scale, shift, side=None, order=(3, 4, 1, 2, 0, 5)):
            m = [None] * 6
            for q, i in enumerate(order):
                lhs = jnp.concatenate([pltpu.bitcast(ts[slot, i, kc], BF) for kc in range(KC)], axis=1)
                words = wu[0, nb] if i == 0 else wu[2, nb] if i == 5 else gs[nb].bitcast(U32)[i - 1]
                m[i] = jnp.dot(lhs, pltpu.bitcast(words, BF), preferred_element_type=F32)
                for f in (side[q] if side else ()):
                    f(m[i])
            sc = scale[:, nb * L:(nb + 1) * L]
            sh = shift[:, nb * L:(nb + 1) * L]
            s1, e1 = m[1] + m[2], m[1] - m[2]
            s2, e2 = m[3] + m[4], m[3] - m[4]
            h0 = s1 * (sc * CA) + (s2 * (sc * CB) + (m[0] * sc + sh))
            h1 = e1 * (sc * (CA * PA)) + (e2 * (sc * (CB * PB)) + sh)
            h2 = s1 * (sc * (CA * PA**2)) + (s2 * (sc * (CB * PB**2)) + sh)
            h3 = e1 * (sc * (CA * PA**3)) + (e2 * (sc * (CB * PB**3)) + (m[5] * sc + sh))

            def act(h):
                return h * jnp.tanh(h) + h
            ov = (os0.bitcast(U32).at[nb] if (isinstance(oslot, int) and oslot == 2)
                  else os_.bitcast(U32).at[oslot, nb])
            ov[pl.ds(0, n, stride=2), :] = _pair(act(h0), act(h1))
            ov[pl.ds(1, n, stride=2), :] = _pair(act(h2), act(h3))

        zrows = jnp.zeros((16, L), BF)
        for s in range(2):
            for kc in range(KC):
                xs[s, kc, pl.ds(0, 16), :] = zrows
                xs[s, kc, pl.ds(XR - 16, 16), :] = zrows
        x0 = x_copies(0, 0, True)
        x1 = x_copies(1, 1, True)
        for c in w_copies(0) + x0:
            c.start()
        for nb in (1, 2):
            for c in w_copies(nb):
                c.start(priority=1)
        mean_v = mean_ref[...].astype(F32).reshape(1, C)
        var_v = var_ref[...].astype(F32).reshape(1, C)
        g_v = g_ref[...].astype(F32).reshape(1, C)
        b_v = b_ref[...].astype(F32).reshape(1, C)
        sc_full = g_v * (1.0 / jnp.sqrt(var_v + EPS))
        scale = 0.5 * sc_full
        shift = 0.5 * (b_v - mean_v * sc_full)

        for c in w_copies(0):
            c.wait()
        for f in g_pieces(0):
            f()
        for kc in range(KC):
            x0[kc].wait()
            for f in x_pieces(0, 0, kc):
                f()

        slots = [[] for _ in range(6 * KC)]
        for nb in range(1, KC):
            def sync(dep=None, nb=nb):
                for c in w_copies(nb):
                    c.wait()
                if nb + 2 < KC:
                    for c in w_copies(nb + 2):
                        c.start(priority=1)
                if nb + 2 == KC:
                    for c in x1:
                        c.start(priority=1)
                if nb + 1 == KC:
                    for c in x_copies(2, 0):
                        c.start(priority=1)
            d0 = 6 * nb - 4
            slots[d0].append(sync)
            for q, fs in enumerate(_spread(g_pieces(nb), 6)):
                slots[d0 + q] += fs
        for nb in range(KC):
            step(0, 2 if nb < H else 0, nb, scale, shift, slots[6 * nb:6 * nb + 6], (0, 5, 1, 2, 3, 4))
        for nb in range(KC):
            o_copy(0, 2 if nb < H else 0, nb).start()
        for kc in range(KC):
            x1[kc].wait()
            for f in x_pieces(1, 1, kc):
                f()
        for nb in range(H):
            step(1, 0, nb, scale, shift)
            o_copy(1, 0, nb).start()

        def body(t, last=False):
            slot = t % 2
            nslot = 1 - slot
            if not last:
                x_wait_all(nslot)
                pieces = _spread([f for kc in range(KC) for f in x_pieces(t + 1, nslot, kc)], KC - H)
            for nb in range(H, KC):
                side = None
                if not last:
                    fs = list(pieces[nb - H])
                    if nb == min(H + 2, KC - 1):
                        def prefetch(dep=None):
                            for c in x_copies(jnp.minimum(t + 2, T - 1), slot):
                                c.start()
                        fs = [prefetch] + fs
                    side = _spread(fs, 6)
                step(slot, slot, nb, scale, shift, side)
                o_copy(t, slot, nb).start()
            if not last:
                for nb in range(H):
                    step(nslot, slot, nb, scale, shift)
                    o_copy(t + 1, slot, nb).start()
                o_wait_all(nslot)

        pl.loop(1, T - 1)(body)
        body(T - 1, last=True)
        x_wait_all(T % 2)
        for nb in range(H):
            o_copy(0, 2, nb).wait()
        o_wait_all(T % 2)
        for nb in range(H, KC):
            o_copy(T - 1, (T - 1) % 2, nb).wait()

    vec = pl.BlockSpec((C,), lambda: (0,))
    hbm = pl.BlockSpec(memory_space=pl.ANY)
    return pl.pallas_call(
        kernel,
        in_specs=[hbm, hbm, vec, vec, vec, vec],
        out_specs=hbm,
        out_shape=jax.ShapeDtypeStruct((B, S, C), x.dtype),
        scratch_shapes=[
            pltpu.VMEM((2, KC, XR, L), BF),
            pltpu.VMEM((2, 6, KC, n // 2, L), U32),
            pltpu.VMEM((3, KC, C, L), BF),
            pltpu.VMEM((2, KC, R + 16, L), BF),
            pltpu.VMEM((H, R + 16, L), BF),
            pltpu.SemaphoreType.DMA((2, KC)),
            pltpu.SemaphoreType.DMA((2,)),
            pltpu.SemaphoreType.DMA((KC,)),
            pltpu.SemaphoreType.DMA((3,)),
        ] + [pltpu.VMEM((4, C, L), BF) for _ in range(KC)],
        compiler_params=pltpu.CompilerParams(vmem_limit_bytes=100 * 1024 * 1024,
                                             disable_bounds_checks=True),
    )(x, w, mean, var, g, b)


@jax.jit
def pallas_standalone__batchnorm__prompt_kernel(
    x: jax.Array,
    w: jax.Array,
    mean: jax.Array,
    var: jax.Array,
    g: jax.Array,
    b: jax.Array,
):
    return _conv_bn_silu(x, w, mean, var, g, b)
```

```python
import functools

import numpy as np
import jax
import jax.numpy as jnp
import jax.experimental.pallas as pl
import jax.experimental.pallas.tpu as pltpu

BF = jnp.bfloat16
F32 = jnp.float32
U32 = jnp.uint32
L = 128
PA, PB = 2.0 / 3.0, 1.5
CA = 1.0 / (2 * PA**2 * (PA**2 - PB**2))
CB = 1.0 / (PA**2 * 2 * PB**2 * (PB**2 - PA**2))
EPS = 1e-5
HI_HALF = np.uint32(0xFFFF0000)


def _lo(u):
    return pltpu.bitcast(u << 16, F32)


def _hi(u):
    return pltpu.bitcast(u & HI_HALF, F32)


def _pair(lo, hi):
    def rounded(v):
        return pltpu.bitcast(v.astype(BF).astype(F32), U32)
    return (rounded(lo) >> 16) | rounded(hi)


def _spread(fs, nslots):
    out = [[] for _ in range(nslots)]
    for q, f in enumerate(fs):
        out[q * nslots // len(fs)].append(f)
    return out


def _conv_bn_silu(x, w, mean, var, g, b, *, R=512, GR=32, TR=64, H=2):
    B, S, C = x.shape
    n = R // 4
    nt = S // R
    T = B * nt
    KC = C // L
    XR = 16 + R + 32 + 16
    assert S % R == 0 and nt >= 2 and T >= 3 and n % TR == 0 and C % GR == 0
    assert KC >= 4 and 1 <= H < KC

    def kernel(x_hbm, w_hbm, mean_ref, var_ref, g_ref, b_ref, o_hbm,
               xs, ts, wr, os_, os0, xsem0, xsem, wsem, osem, *gs):
        xu = xs.bitcast(U32)
        tu = ts.bitcast(U32)
        wu = wr.bitcast(U32)

        def tile_pos(t):
            bi = t // nt
            i = t % nt
            start = jnp.clip(i * R - 16, 0, S - R - 32)
            return bi, i, pl.multiple_of(start, 16)

        def x_copies(t, slot, per_block_sem=False):
            bi, _, start = tile_pos(t)
            return [pltpu.make_async_copy(x_hbm.at[bi, pl.ds(start, R + 32), pl.ds(kc * L, L)],
                                          xs.at[slot, kc, pl.ds(16, R + 32), :],
                                          xsem0.at[slot, kc] if per_block_sem else xsem.at[slot])
                    for kc in range(KC)]

        def x_wait_all(slot):
            win = xs.at[slot, :, pl.ds(16, R + 32), :]
            pltpu.make_async_copy(win, win, xsem.at[slot]).wait()

        def w_copies(nb):
            return [pltpu.make_async_copy(w_hbm.at[k, :, pl.ds(nb * L, L)], wr.at[k, nb], wsem.at[nb])
                    for k in range(3)]

        def o_stage(oslot, nb):
            return (os0.at[nb, pl.ds(0, R), :] if (isinstance(oslot, int) and oslot == 2)
                    else os_.at[oslot, nb, pl.ds(0, R), :])

        def o_copy(t, oslot, nb):
            bi = t // nt
            i = t % nt
            return pltpu.make_async_copy(
                o_stage(oslot, nb),
                o_hbm.at[bi, pl.ds(pl.multiple_of(i * R, R), R), pl.ds(nb * L, L)], osem.at[oslot])

        def o_wait_all(oslot):
            blocks = os_.at[oslot, :, pl.ds(0, R), :]
            pltpu.make_async_copy(blocks, blocks, osem.at[oslot]).wait()

        def x_piece(t, slot, kc, j0, dep=None):
            _, i, start = tile_pos(t)
            off = pl.multiple_of((i * R - start) // 2, 8)
            xv = xu.at[slot, kc, pl.ds(off, R // 2 + 16), :]

            def ld(o):
                return xv[pl.ds(8 + 2 * j0 + o, TR, stride=2), :]
            we, wo, wp, wn = ld(0), ld(1), ld(-1), ld(2)
            d0, d1, d2, d3, d4, d5 = _hi(wp), _lo(we), _hi(we), _lo(wo), _hi(wo), _lo(wn)
            u = (PB * PB) * d2
            v = (PA * PA) * d2
            pa = d4 - u
            pb = d4 - v
            qa = PA * d3 - PB * d1
            qb = PB * d3 - PA * d1
            r = pl.ds(j0, TR)
            ts[slot, 0, kc, r] = ((d0 - u) + pb).astype(BF)
            ts[slot, 1, kc, r] = (pa + qa).astype(BF)
            ts[slot, 2, kc, r] = (pa - qa).astype(BF)
            ts[slot, 3, kc, r] = (pb + qb).astype(BF)
            ts[slot, 4, kc, r] = (pb - qb).astype(BF)
            ts[slot, 5, kc, r] = ((d1 + d5) - (PA * PA + PB * PB) * d3).astype(BF)

        def x_pieces(t, slot, kc):
            return [functools.partial(x_piece, t, slot, kc, j0) for j0 in range(0, n, TR)]

        def g_piece(nb, r0, dep=None):
            r = pl.ds(r0, GR)
            g0, g1, g2 = (wr[k, nb, r].astype(F32) for k in range(3))
            c2, c1 = PA * PA, PA
            if dep is not None:
                z = (pltpu.bitcast(dep[0:8, :], U32) >> 16) >> 16

                def cst(val):
                    c = pltpu.bitcast(pltpu.bitcast(jnp.full((8, L), val, F32), U32) | z, F32)
                    return jnp.tile(c, (GR // 8, 1))
                c2, c1 = cst(PA * PA), cst(PA)
            ea = g0 + g2 * c2
            eb = g0 * c2 + g2
            o = g1 * c1
            gs[nb][0, r] = (ea + o).astype(BF)
            gs[nb][1, r] = (ea - o).astype(BF)
            gs[nb][2, r] = (eb + o).astype(BF)
            gs[nb][3, r] = (eb - o).astype(BF)

        def g_pieces(nb):
            return [functools.partial(g_piece, nb, r0) for r0 in range(0, C, GR)]

        def step(slot, oslot, nb, scale, shift, side=None, order=(1, 2, 0, 3, 4, 5)):
            m = [None] * 6
            for q, i in enumerate(order):
                lhs = jnp.concatenate([pltpu.bitcast(tu[slot, i, kc], BF) for kc in range(KC)], axis=1)
                words = wu[0, nb] if i == 0 else wu[2, nb] if i == 5 else gs[nb].bitcast(U32)[i - 1]
                m[i] = jnp.dot(lhs, pltpu.bitcast(words, BF), preferred_element_type=F32)
                for f in (side[q] if side else ()):
                    f(m[i])
            sc = scale[:, nb * L:(nb + 1) * L]
            sh = shift[:, nb * L:(nb + 1) * L]
            s1, e1 = m[1] + m[2], m[1] - m[2]
            s2, e2 = m[3] + m[4], m[3] - m[4]
            h0 = s1 * (sc * CA) + (s2 * (sc * CB) + (m[0] * sc + sh))
            h1 = e1 * (sc * (CA * PA)) + (e2 * (sc * (CB * PB)) + sh)
            h2 = s1 * (sc * (CA * PA**2)) + (s2 * (sc * (CB * PB**2)) + sh)
            h3 = e1 * (sc * (CA * PA**3)) + (e2 * (sc * (CB * PB**3)) + (m[5] * sc + sh))

            def act(h):
                return h * jnp.tanh(h) + h
            ov = (os0.bitcast(U32).at[nb] if (isinstance(oslot, int) and oslot == 2)
                  else os_.bitcast(U32).at[oslot, nb])
            ov[pl.ds(0, n, stride=2), :] = _pair(act(h0), act(h1))
            ov[pl.ds(1, n, stride=2), :] = _pair(act(h2), act(h3))

        zrows = jnp.zeros((16, L), BF)
        for s in range(2):
            for kc in range(KC):
                xs[s, kc, pl.ds(0, 16), :] = zrows
                xs[s, kc, pl.ds(XR - 16, 16), :] = zrows
        x0 = x_copies(0, 0, True)
        x1 = x_copies(1, 1, True)
        for c in w_copies(0) + x0:
            c.start()
        for nb in (1, 2):
            for c in w_copies(nb):
                c.start(priority=1)
        mean_v = mean_ref[...].astype(F32).reshape(1, C)
        var_v = var_ref[...].astype(F32).reshape(1, C)
        g_v = g_ref[...].astype(F32).reshape(1, C)
        b_v = b_ref[...].astype(F32).reshape(1, C)
        sc_full = g_v * (1.0 / jnp.sqrt(var_v + EPS))
        scale = 0.5 * sc_full
        shift = 0.5 * (b_v - mean_v * sc_full)

        for c in w_copies(0):
            c.wait()
        for f in g_pieces(0):
            f()
        for kc in range(KC):
            x0[kc].wait()
            for f in x_pieces(0, 0, kc):
                f()

        slots = [[] for _ in range(6 * KC)]
        for nb in range(1, KC):
            def sync(dep=None, nb=nb):
                for c in w_copies(nb):
                    c.wait()
                if nb + 2 < KC:
                    for c in w_copies(nb + 2):
                        c.start(priority=1)
                if nb + 2 == KC:
                    for c in x1:
                        c.start(priority=1)
                if nb + 1 == KC:
                    for c in x_copies(2, 0):
                        c.start(priority=1)
            d0 = 6 * nb - 4
            slots[d0].append(sync)
            for q, fs in enumerate(_spread(g_pieces(nb), 6)):
                slots[d0 + q] += fs
        for nb in range(KC):
            step(0, 2 if nb < H else 0, nb, scale, shift, slots[6 * nb:6 * nb + 6], (0, 5, 1, 2, 3, 4))
        for nb in range(KC):
            o_copy(0, 2 if nb < H else 0, nb).start()
        for kc in range(KC):
            x1[kc].wait()
            for f in x_pieces(1, 1, kc):
                f()
        for nb in range(H):
            step(1, 0, nb, scale, shift)
            o_copy(1, 0, nb).start()

        def body(t, last=False):
            slot = t % 2
            nslot = 1 - slot
            if not last:
                x_wait_all(nslot)
                pieces = _spread([f for kc in range(KC) for f in x_pieces(t + 1, nslot, kc)], KC - H)
            for nb in range(H, KC):
                side = None
                if not last:
                    fs = list(pieces[nb - H])
                    if nb == min(H + 2, KC - 1):
                        def prefetch(dep=None):
                            for c in x_copies(jnp.minimum(t + 2, T - 1), slot):
                                c.start()
                        fs = [prefetch] + fs
                    side = _spread(fs, 6)
                step(slot, slot, nb, scale, shift, side)
                o_copy(t, slot, nb).start()
            if not last:
                for nb in range(H):
                    step(nslot, slot, nb, scale, shift)
                    o_copy(t + 1, slot, nb).start()
                o_wait_all(nslot)

        pl.loop(1, T - 1)(body)
        body(T - 1, last=True)
        x_wait_all(T % 2)
        for nb in range(H):
            o_copy(0, 2, nb).wait()
        o_wait_all(T % 2)
        for nb in range(H, KC):
            o_copy(T - 1, (T - 1) % 2, nb).wait()

    vec = pl.BlockSpec((C,), lambda: (0,))
    hbm = pl.BlockSpec(memory_space=pl.ANY)
    return pl.pallas_call(
        kernel,
        in_specs=[hbm, hbm, vec, vec, vec, vec],
        out_specs=hbm,
        out_shape=jax.ShapeDtypeStruct((B, S, C), x.dtype),
        scratch_shapes=[
            pltpu.VMEM((2, KC, XR, L), BF),
            pltpu.VMEM((2, 6, KC, n, L), BF),
            pltpu.VMEM((3, KC, C, L), BF),
            pltpu.VMEM((2, KC, R + 16, L), BF),
            pltpu.VMEM((H, R + 16, L), BF),
            pltpu.SemaphoreType.DMA((2, KC)),
            pltpu.SemaphoreType.DMA((2,)),
            pltpu.SemaphoreType.DMA((KC,)),
            pltpu.SemaphoreType.DMA((3,)),
        ] + [pltpu.VMEM((4, C, L), BF) for _ in range(KC)],
        compiler_params=pltpu.CompilerParams(vmem_limit_bytes=100 * 1024 * 1024,
                                             disable_bounds_checks=True),
    )(x, w, mean, var, g, b)


@jax.jit
def pallas_standalone__batchnorm__prompt_kernel(
    x: jax.Array,
    w: jax.Array,
    mean: jax.Array,
    var: jax.Array,
    g: jax.Array,
    b: jax.Array,
):
    return _conv_bn_silu(x, w, mean, var, g, b)
```
